```python
import os as _os
_os.environ.setdefault("JAX_PLATFORMS", "cpu")
import jax
import jax.numpy as jnp

def _softmax(x, axis=-1):
    return jax.nn.softmax(x, axis=axis)
def _gelu(x):
    return jax.nn.gelu(x, approximate=True)
def _silu(x):
    return jax.nn.silu(x)
def _sigmoid(x):
    return jax.nn.sigmoid(x)
def _layernorm(x, axis=-1, eps=1e-5):
    m = jnp.mean(x, axis=axis, keepdims=True)
    v = jnp.var(x, axis=axis, keepdims=True)
    return (x - m) / jnp.sqrt(v + eps)
def _scatter_add(tgt, idx, src, axis=0):
    return tgt.at[idx].add(src)
def _segment_sum(src, seg, n):
    return jax.ops.segment_sum(src, seg, n)
class _Rng:
    def __init__(self, key):
        self._k = key
    def _next(self):
        self._k, sub = jax.random.split(self._k)
        return sub
    def normal(self, shape):
        return jax.random.normal(self._next(), shape, dtype=jnp.bfloat16)
    def randint(self, lo, hi, shape):
        return jax.random.randint(self._next(), shape, lo, hi, dtype=jnp.int32)
    def uniform(self, shape, lo=0.0, hi=1.0):
        return jax.random.uniform(self._next(), shape, jnp.bfloat16, lo, hi)
    def permutation(self, n):
        return jax.random.permutation(self._next(), n)


kernel_name = 'standalone__channel_attn_cbam__vision'

def setup_inputs():
    _rng = _Rng(jax.random.key(int.from_bytes(__import__("os").urandom(4), "little")))
    _w = (lambda a: (lambda t: t.astype(jnp.bfloat16) if jnp.issubdtype(t.dtype, jnp.floating) else t)(jnp.asarray(a)))
    H = W = 224
    C = 192
    r = max(C // 4, 1)
    return {
        "x": _w((lambda *s: _rng.normal(s) * 0.2)(1, H, W, C) + (lambda *s: _rng.normal(s) * 0.2)(1, 1, 1, C) * 2.0),
        "w1": _w((lambda *s: _rng.normal(s) * 0.2)(C, r)),
        "w2": _w((lambda *s: _rng.normal(s) * 0.2)(r, C)),
    }

def reference(x, w1, w2):
    B, H, W, C = x.shape
    xf = x.reshape(B, H * W, C)
    gap = jnp.mean(xf, 1)
    gmp = jnp.amax(xf, 1)
    h_a = gap @ w1
    h_a = h_a * (lambda x, dt: x.astype(dt))(h_a > 0, h_a.dtype)
    h_m = gmp @ w1
    h_m = h_m * (lambda x, dt: x.astype(dt))(h_m > 0, h_m.dtype)
    scale = _sigmoid(h_a @ w2 + h_m @ w2)
    return x * scale[:, None, None, :]
```

```python
import jax
import jax.numpy as jnp
from jax import lax
import jax.experimental.pallas as pl
import jax.experimental.pallas.tpu as pltpu


@jax.jit
def pallas_standalone__channel_attn_cbam__vision_kernel(
    x: jax.Array,
    w1: jax.Array,
    w2: jax.Array,
):
    _, H, W, C = x.shape
    R = w1.shape[1]
    G = C // 8
    B2, cc, K = 6144, 16, 4
    tail = (128, 64, 24, 8)
    A2 = H * C // B2
    J = B2 // cc
    NF = G - 1

    def kern(x_hbm, w1t_hbm, w2_hbm, o_hbm, buf, wbuf, w1d, w2d, sc_ref, rsem, wsem):
        def rd_full(g, slot):
            s = (slice(None), pl.ds(pl.multiple_of(g * 8, 8), 8))
            return pltpu.make_async_copy(x_hbm.at[s], buf.at[s], rsem.at[slot])

        def rd_tail(t):
            s = (pl.ds(sum(tail[:t]), tail[t]), pl.ds(NF * 8, 8))
            return pltpu.make_async_copy(x_hbm.at[s], buf.at[s], rsem.at[(NF + t) % K])

        cw1 = pltpu.make_async_copy(w1t_hbm, wbuf.at[0], wsem)
        cw2 = pltpu.make_async_copy(w2_hbm, wbuf.at[1], wsem)
        rd_full(0, 0).start()
        cw1.start()
        cw2.start()

        @pl.loop(1, K)
        def _(g):
            rd_full(g, g).start()

        cw1.wait()
        cw2.wait()
        for k, dst in ((0, w1d), (1, w2d)):
            w = wbuf[k].astype(jnp.float32)
            z = jnp.zeros((64 - R, C), jnp.float32)
            w = jnp.concatenate([w, z, w, z], axis=0)
            w = jnp.concatenate([w, jnp.zeros((128, 256 - C), jnp.float32)], axis=1)
            dst[...] = w.T[:C]
        lane = lax.broadcasted_iota(jnp.int32, (8, 128), 1)

        def accum(g, h0, n, carry):
            u = n if n <= 32 else 16

            def body(i, carry):
                carry = list(carry)
                for k in range(u):
                    s0, s1, m0, m1 = carry[k % 2]
                    v = buf[h0 + i * u + k, pl.ds(g * 8, 8), :].astype(jnp.float32)
                    a, b = v[:, :128], v[:, 128:]
                    carry[k % 2] = (s0 + a, s1 + b, jnp.maximum(m0, a), jnp.maximum(m1, b))
                return tuple(carry)

            if n == u:
                return body(0, carry)
            return lax.fori_loop(0, n // u, body, carry)

        def init():
            one = (jnp.zeros((8, 128), jnp.float32), jnp.zeros((8, W - 128), jnp.float32),
                   jnp.full((8, 128), -jnp.inf, jnp.float32),
                   jnp.full((8, W - 128), -jnp.inf, jnp.float32))
            return (one, one)

        def finish(g, carry, hacc):
            (s0, s1, m0, m1), (t0, t1, n0, n1) = carry
            s = jnp.sum(jnp.concatenate([s0 + t0, s1 + t1], axis=1), axis=1, keepdims=True)
            m = jnp.max(jnp.concatenate([jnp.maximum(m0, n0), jnp.maximum(m1, n1)], axis=1),
                        axis=1, keepdims=True)
            gap = (s / (H * W)).astype(jnp.bfloat16).astype(jnp.float32)
            d = jnp.where(lane < 64, gap, m)
            return hacc + d * w1d[pl.ds(g * 8, 8), :]

        def gbody(g, hacc):
            slot = g % K
            rd_full(g, slot).wait()

            @pl.when(g + K < NF)
            def _():
                rd_full(g + K, slot).start()

            for t in range(min(K, len(tail))):
                @pl.when(g + K == NF + t)
                def _():
                    rd_tail(t).start()
            return finish(g, accum(g, 0, H, init()), hacc)

        hacc = lax.fori_loop(0, NF, gbody, jnp.zeros((8, 128), jnp.float32))
        carry = init()
        for t in range(len(tail)):
            rd_tail(t).wait()
            if t + K < len(tail):
                rd_tail(t + K).start()
            carry = accum(NF, sum(tail[:t]), tail[t], carry)
        hacc = finish(NF, carry, hacc)
        h = jnp.sum(hacc, axis=0, keepdims=True).astype(jnp.bfloat16).astype(jnp.float32)
        h = h * (h > 0).astype(jnp.float32)
        z = jnp.sum(w2d[...] * h, axis=1, keepdims=True)
        sc = jax.nn.sigmoid(z).astype(jnp.bfloat16).astype(jnp.float32)
        sc = jnp.broadcast_to(sc, (C, 128))
        sc_ref[pl.ds(0, C), :] = sc
        sc_ref[pl.ds(C, C), :] = sc

        bv = buf.reshape(A2, B2, W)

        def do_chunk(j0, getscale):
            cache = {}
            for a in range(A2):
                for q in range(cc // 8):
                    off = (a * (B2 // 8) + q) % G
                    if off not in cache:
                        s = getscale(off)
                        cache[off] = jnp.concatenate([s, s[:, :W - 128]], axis=1)
                    r = j0 + q * 8
                    if not isinstance(r, int):
                        r = pl.multiple_of(r, 8)
                    v = bv[a, pl.ds(r, 8), :].astype(jnp.float32)
                    bv[a, pl.ds(r, 8), :] = (v * cache[off]).astype(jnp.bfloat16)
            s = (slice(None), pl.ds(j0, cc))
            pltpu.make_async_copy(bv.at[s], o_hbm.at[s], wsem).start()

        do_chunk(0, lambda off: sc[off * 8:off * 8 + 8])

        def jbody(j, g0):
            do_chunk(pl.multiple_of(j * cc, 8),
                     lambda off: sc_ref[pl.ds(pl.multiple_of((g0 + off) * 8, 8), 8), :])
            g1 = g0 + cc // 8
            return jnp.where(g1 >= G, g1 - G, g1)

        lax.fori_loop(1, J, jbody, (cc // 8) % G)
        pltpu.make_async_copy(bv, o_hbm, wsem).wait()

    xt = x.transpose(0, 1, 3, 2).reshape(H, C, W)
    out = pl.pallas_call(
        kern,
        out_shape=jax.ShapeDtypeStruct((A2, B2, W), x.dtype),
        in_specs=[pl.BlockSpec(memory_space=pl.ANY)] * 3,
        out_specs=pl.BlockSpec(memory_space=pl.ANY),
        scratch_shapes=[
            pltpu.VMEM((H, C, W), x.dtype),
            pltpu.VMEM((2, R, C), w1.dtype),
            pltpu.VMEM((C, 128), jnp.float32),
            pltpu.VMEM((C, 128), jnp.float32),
            pltpu.VMEM((2 * C, 128), jnp.float32),
            pltpu.SemaphoreType.DMA((K,)),
            pltpu.SemaphoreType.DMA(()),
        ],
        compiler_params=pltpu.CompilerParams(vmem_limit_bytes=48 * 1024 * 1024),
    )(xt, w1.T, w2)
    return out.reshape(1, H, C, W).transpose(0, 1, 3, 2)
```

```python
import jax
import jax.numpy as jnp
from jax import lax
import jax.experimental.pallas as pl
import jax.experimental.pallas.tpu as pltpu

_F32 = jnp.float32
_LANES = 128

_A = 7
_HC = 16
_TC = 16
_CC = 16
_LAST = 8
_K = 3
_NP = 4


@jax.jit
def pallas_standalone__channel_attn_cbam__vision_kernel(
    x: jax.Array,
    w1: jax.Array,
    w2: jax.Array,
):
    B, H, W, C = x.shape
    R = w1.shape[1]
    P = H // _A
    CB = C - _TC
    NB = H // _HC
    NK = C // _CC
    assert B == 1 and H == _A * P and P % _HC == 0 and P % _LAST == 0
    assert C % _CC == 0 and C <= 2 * _LANES and R <= _LANES // 2
    assert _LANES < W <= 2 * _LANES
    tail = ((0, 4, 0, P), (4, 2, 0, P), (6, 1, 0, P - _LAST), (6, 1, P - _LAST, _LAST))

    def kernel(x_hbm, w1t_hbm, w2_hbm, o_hbm, buf, wbuf, w1d, w2d, acc, scale, sem):
        def bulk_pos(i):
            return i // (P // _HC), (i % (P // _HC)) * _HC

        def read_bulk(i):
            a, p0 = bulk_pos(i)
            s = (a, pl.ds(p0, _HC), pl.ds(0, CB))
            return pltpu.make_async_copy(x_hbm.at[s], buf.at[s], sem.at[i % _K])

        def read_tail(t):
            a0, na, p0, n = tail[t]
            s = (pl.ds(a0, na), pl.ds(p0, n), pl.ds(CB, _TC))
            return pltpu.make_async_copy(x_hbm.at[s], buf.at[s], sem.at[(NB + t) % _K])

        def pool(r, nr, a, p0, n, carry):
            carry = list(carry)
            for k in range(n):
                s, m = carry[k % len(carry)]
                v = buf[a, p0 + k, pl.ds(r, nr), :].astype(_F32)
                carry[k % len(carry)] = (s + v, jnp.maximum(m, v))
            return tuple(carry)

        def pool_init(nr):
            return jnp.zeros((nr, W), _F32), jnp.full((nr, W), -jnp.inf, _F32)

        def layer1(r, s, m):
            n = s.shape[0]
            gap = jnp.sum(s, axis=1, keepdims=True) / (H * W)
            gap = gap.astype(x.dtype).astype(_F32)
            gmp = jnp.max(m, axis=1, keepdims=True)
            lane = lax.broadcasted_iota(jnp.int32, (n, _LANES), 1)
            d = jnp.where(lane < _LANES // 2, gap, gmp) * w1d[pl.ds(r, n), :]
            return jnp.sum(d.reshape(n // 8, 8, _LANES), axis=0)

        cw1 = pltpu.make_async_copy(w1t_hbm, wbuf.at[0], sem.at[_K - 1])
        cw2 = pltpu.make_async_copy(w2_hbm, wbuf.at[1], sem.at[_K - 1])
        read_bulk(0).start()
        cw1.start()
        cw2.start()
        pl.delay(1)
        for i in range(1, _K - 1):
            read_bulk(i).start()
        acc[0], acc[1] = pool_init(CB)
        cw1.wait()
        cw2.wait()
        read_bulk(_K - 1).start()

        for k, dst in enumerate((w1d, w2d)):
            w = wbuf[k].astype(_F32)
            gap_rows = jnp.zeros((_LANES // 2 - R, C), _F32)
            w = jnp.concatenate([w, gap_rows, w, gap_rows], axis=0)
            w = jnp.concatenate([w, jnp.zeros((_LANES, 2 * _LANES - C), _F32)], axis=1)
            dst[...] = w.T[:C]

        @pl.loop(0, NB)
        def _(i):
            read_bulk(i).wait()

            @pl.when(i + _K < NB)
            def _():
                read_bulk(i + _K).start()

            for t in range(_K):
                @pl.when(i + _K == NB + t)
                def _():
                    read_tail(t).start()

            a, p0 = bulk_pos(i)

            @pl.loop(0, CB // 8)
            def _(g):
                r = pl.multiple_of(g * 8, 8)
                old = (acc[0, pl.ds(r, 8), :], acc[1, pl.ds(r, 8), :])
                (s0, m0), (s1, m1) = pool(r, 8, a, p0, _HC, (old, pool_init(8)))
                acc[0, pl.ds(r, 8), :] = s0 + s1
                acc[1, pl.ds(r, 8), :] = jnp.maximum(m0, m1)

        hidden = layer1(0, acc[0], acc[1])

        def tail_body(i, carry):
            for t in range(len(tail) - 1):
                @pl.when(i == tail[t][0] * (P // _LAST))
                def _():
                    read_tail(t).wait()
                    if t + _K < len(tail):
                        read_tail(t + _K).start()

            return pool(CB, _TC, i // (P // _LAST), (i % (P // _LAST)) * _LAST, _LAST, carry)

        carry = lax.fori_loop(0, H // _LAST - 1, tail_body, (pool_init(_TC),))
        read_tail(len(tail) - 1).wait()
        carry = pool(CB, _TC, _A - 1, P - _LAST, _LAST, carry)
        hidden = hidden + layer1(CB, *carry[0])

        h = jnp.sum(hidden, axis=0, keepdims=True).astype(x.dtype).astype(_F32)
        h = h * (h > 0).astype(_F32)
        z = jnp.sum(w2d[...] * h, axis=1, keepdims=True)
        z = jnp.broadcast_to(z, (C, _LANES))

        def gate(z):
            return jax.nn.sigmoid(z).astype(x.dtype).astype(_F32)

        def write_chunk(p, c0, sc):
            sc = jnp.concatenate([sc, sc[:, :W - _LANES]], axis=1)
            for a in range(_A):
                v = buf[a, p, pl.ds(c0, _CC), :].astype(_F32)
                buf[a, p, pl.ds(c0, _CC), :] = (v * sc).astype(x.dtype)
            s = (slice(None), p, pl.ds(c0, _CC))
            pltpu.make_async_copy(buf.at[s], o_hbm.at[s], sem.at[0]).start()

        for k in range(_NP):
            sc = gate(z[k * _CC:(k + 1) * _CC])
            scale[pl.ds(k * _CC, _CC), :] = sc
            write_chunk(0, k * _CC, sc)
            if k == 0:
                pl.delay(1)
        scale[pl.ds(_NP * _CC, C - _NP * _CC), :] = gate(z[_NP * _CC:])

        def write_body(_, pk):
            p, k = pk
            c0 = pl.multiple_of(k * _CC, _CC)
            write_chunk(p, c0, scale[pl.ds(c0, _CC), :])
            wrap = k == NK - 1
            return jnp.where(wrap, p + 1, p), jnp.where(wrap, 0, k + 1)

        lax.fori_loop(_NP, P * NK, write_body, (0, _NP))
        pltpu.make_async_copy(buf, o_hbm, sem.at[0]).wait()

    hbm = pl.BlockSpec(memory_space=pl.ANY)
    out = pl.pallas_call(
        kernel,
        out_shape=jax.ShapeDtypeStruct((_A, P, C, W), x.dtype),
        in_specs=[hbm, hbm, hbm],
        out_specs=hbm,
        scratch_shapes=[
            pltpu.VMEM((_A, P, C, W), x.dtype),
            pltpu.VMEM((2, R, C), w1.dtype),
            pltpu.VMEM((C, _LANES), _F32),
            pltpu.VMEM((C, _LANES), _F32),
            pltpu.VMEM((2, CB, W), _F32),
            pltpu.VMEM((C, _LANES), _F32),
            pltpu.SemaphoreType.DMA((_K,)),
        ],
        compiler_params=pltpu.CompilerParams(vmem_limit_bytes=48 * 1024 * 1024),
    )(x.transpose(0, 1, 3, 2).reshape(_A, P, C, W), w1.T, w2)
    return out.reshape(1, H, C, W).transpose(0, 1, 3, 2)
```
